```python
import os as _os
_os.environ.setdefault("JAX_PLATFORMS", "cpu")
import jax
import jax.numpy as jnp

def _softmax(x, axis=-1):
    return jax.nn.softmax(x, axis=axis)
def _gelu(x):
    return jax.nn.gelu(x, approximate=True)
def _silu(x):
    return jax.nn.silu(x)
def _sigmoid(x):
    return jax.nn.sigmoid(x)
def _layernorm(x, axis=-1, eps=1e-5):
    m = jnp.mean(x, axis=axis, keepdims=True)
    v = jnp.var(x, axis=axis, keepdims=True)
    return (x - m) / jnp.sqrt(v + eps)
def _scatter_add(tgt, idx, src, axis=0):
    return tgt.at[idx].add(src)
def _segment_sum(src, seg, n):
    return jax.ops.segment_sum(src, seg, n)
class _Rng:
    def __init__(self, key):
        self._k = key
    def _next(self):
        self._k, sub = jax.random.split(self._k)
        return sub
    def normal(self, shape):
        return jax.random.normal(self._next(), shape, dtype=jnp.bfloat16)
    def randint(self, lo, hi, shape):
        return jax.random.randint(self._next(), shape, lo, hi, dtype=jnp.int32)
    def uniform(self, shape, lo=0.0, hi=1.0):
        return jax.random.uniform(self._next(), shape, jnp.bfloat16, lo, hi)
    def permutation(self, n):
        return jax.random.permutation(self._next(), n)


kernel_name = 'gated_mix__mha_block__linear_kernel_hedgehog__prompt'

def setup_inputs():
    _rng = _Rng(jax.random.key(int.from_bytes(__import__("os").urandom(4), "little")))
    _w = (lambda a: (lambda t: t.astype(jnp.bfloat16) if jnp.issubdtype(t.dtype, jnp.floating) else t)(jnp.asarray(a)))
    def _A_setup():
        B, S, D, H = 1, 2048, 640, 32
        return {
            "x": _w((lambda *s: _rng.normal(s) * 0.05)(B, S, D)),
            "wqkv": _w((lambda *s: _rng.normal(s) * 0.4)(D, 3 * D)),
            "wo": _w((lambda *s: _rng.normal(s) * 0.05)(D, D)),
        }
    _A_in = _A_setup()

    def _B_setup():
        B, S, D, H = 1, 2048, 640, 32
        Dh = D // H
        return {
            "x": _w((lambda *s: _rng.normal(s) * 0.05)(B, S, D)),
            "wqkv": _w((lambda *s: _rng.normal(s) * 0.8)(D, 3 * D)),
            "w_phi": _w((lambda *s: _rng.normal(s) * 0.8)(H, Dh, Dh) * (Dh ** -0.5)),
            "wo": _w((lambda *s: _rng.normal(s) * 0.05)(D, D)),
        }
    _B_in = _B_setup()

    return {
        "A_x": _A_in["x"],
        "A_wqkv": _A_in["wqkv"],
        "A_wo": _A_in["wo"],
        "B_x": _B_in["x"],
        "B_wqkv": _B_in["wqkv"],
        "B_w_phi": _B_in["w_phi"],
        "B_wo": _B_in["wo"],
        "gate_w": _w((lambda *s: _rng.normal(s) * 0.05)(640) * 16.0),
    }

def reference(A_x, A_wqkv, A_wo, B_x, B_wqkv, B_w_phi, B_wo, gate_w):
    def _A_ref(x, wqkv, wo):
        B, S, D = x.shape
        H = 32
        Dh = D // H
        qkv = (lambda x, *d: x.transpose(*d))((x @ wqkv).reshape(B, S, 3, H, Dh), 2, 0, 3, 1, 4)
        q, k, v = qkv[0], qkv[1], qkv[2]
        scores = jnp.einsum("bhqd,bhkd->bhqk", q, k) * (Dh ** -0.5)
        p = _softmax(scores, axis=-1)
        o = jnp.einsum("bhqk,bhkd->bhqd", p, v)
        return (lambda x, *d: x.transpose(*d))(o, 0, 2, 1, 3).reshape(B, S, D) @ wo

    def _B_ref(x, wqkv, w_phi, wo):
        B, S, D = x.shape
        H = 32; Dh = D // H
        qkv = (lambda x, *d: x.transpose(*d))((x @ wqkv).reshape(B, S, 3, H, Dh), 2, 0, 3, 1, 4)
        q, k, v = qkv[0], qkv[1], qkv[2]
        pq = jnp.einsum("bhsd,hdf->bhsf", q, w_phi)
        pk = jnp.einsum("bhsd,hdf->bhsf", k, w_phi)
        phi_q = jnp.concatenate([_softmax(pq, axis=-1), _softmax(-pq, axis=-1)], axis=-1)
        phi_k = jnp.concatenate([_softmax(pk, axis=-1), _softmax(-pk, axis=-1)], axis=-1)
        kv = jnp.einsum("bhsf,bhsd->bhfd", phi_k, v)
        z  = jnp.einsum("bhsf->bhf", phi_k)
        num = jnp.einsum("bhqf,bhfd->bhqd", phi_q, kv)
        den = jnp.einsum("bhqf,bhf->bhq", phi_q, z)[..., None] + 1e-6
        o = num / den
        return (lambda x, *d: x.transpose(*d))(o, 0, 2, 1, 3).reshape(B, S, D) @ wo

    x = A_x
    g = _sigmoid((x * gate_w).sum(-1, keepdims=True))
    a = _A_ref(x, A_wqkv, A_wo)
    b = _B_ref(x, B_wqkv, B_w_phi, B_wo)
    return g * a + (1 - g) * b
```

```python
import math

import jax
import jax.numpy as jnp
from jax import lax
import jax.experimental.pallas as pl
import jax.experimental.pallas.tpu as pltpu

F32 = jnp.float32
BF16 = jnp.bfloat16
U32 = jnp.uint32

S = 2048
D = 640
H = 32
DH = 20
LOG2E = math.log2(math.e)
QSCALE = (DH ** -0.5) * LOG2E

WIN = (0, 120, 240, 360, 480, 512)
RN = ((0, 144), (112, 272), (240, 400), (368, 528), (496, 640))

TQ = 512
KC = 128
LAG = 2
HPI = 2
NQ = S // TQ
NC = S // KC
TB = S // (H // HPI)
TP = 256
TF = 256

SAFE_LOG2 = 64.0
V_HI = 2.0 ** 40
V_LO = 2.0 ** -20

NN = (((1,), (0,)), ((), ()))
NT = (((1,), (1,)), ((), ()))


def _dot(a, b, dims=NN):
    return lax.dot_general(a, b, dims, preferred_element_type=F32)


def _iota(shape, dim):
    return lax.broadcasted_iota(jnp.int32, shape, dim)


def _dual_softmax(x):
    t = x.shape[1]
    x3 = x.reshape(H // 2, 2 * DH, t)
    is_a = _iota(x3.shape, 1) < DH
    inf = jnp.float32(jnp.inf)

    def seg(op, fill, v):
        ra = op(jnp.where(is_a, v, fill), axis=1, keepdims=True)
        rb = op(jnp.where(is_a, fill, v), axis=1, keepdims=True)
        return jnp.where(is_a, ra, rb)

    mx = seg(jnp.max, -inf, x3)
    mn = seg(jnp.min, inf, x3)
    ep = jnp.exp2(x3 - mx)
    en = jnp.exp2(mn - x3)
    pp = ep / seg(jnp.sum, 0.0, ep)
    pn = en / seg(jnp.sum, 0.0, en)
    return pp.reshape(D, t), pn.reshape(D, t)


def _scatter_rn(parts):
    pieces = []
    for n in range(5):
        lo, hi = RN[n]
        start = lo if n == 0 else RN[n - 1][1]
        stop = hi if n == 4 else RN[n + 1][0]
        pieces.append(parts[n][start - lo:stop - lo])
        if n < 4:
            nlo = RN[n + 1][0]
            pieces.append(parts[n][nlo - lo:hi - lo] + parts[n + 1][0:hi - nlo])
    return jnp.concatenate(pieces, axis=0)


def _kernel(x_hbm, wa_hbm, woa_hbm, wb_hbm, wphi_hbm, wob_hbm, gw_hbm, out_hbm,
            x_v, wa_v, woa_v, wb_v, wphi_v, wob_v, gw_v, out_v,
            wqk_s, wvt_s, wbt_s, wot_s, t_s,
            q_s, k_s, vt_s, gt_s, at_s,
            qmax_s, kmax_s, vmax_s,
            phiq_s, kvp_s, kvn_s, s_s,
            p0, p1, p2, p3,
            flag_s, in_sems, out_sems):
    pbufs = (p0, p1, p2, p3)

    cps = [pltpu.make_async_copy(src, dst, in_sems.at[i]) for i, (src, dst) in enumerate(
        ((x_hbm.at[0], x_v), (wa_hbm, wa_v), (gw_hbm, gw_v), (wb_hbm, wb_v), (wphi_hbm, wphi_v),
         (woa_hbm, woa_v), (wob_hbm, wob_v)))]
    for c in cps:
        c.start()
    cps[0].wait()
    cps[1].wait()
    cps[2].wait()

    for t in range(6):
        wqk_s[:, t * 128:(t + 1) * 128] = wa_v[:, WIN[t]:WIN[t] + 128]
        wqk_s[:, 768 + t * 128:768 + (t + 1) * 128] = wa_v[:, D + WIN[t]:D + WIN[t] + 128]
    wvt_s[0:D, :] = wa_v[:, 2 * D:3 * D].T
    gw_rows = jnp.where(_iota((16, D), 0) == 0, jnp.broadcast_to(gw_v[...].astype(F32), (16, D)), 0.0)
    wvt_s[D:D + 16, :] = gw_rows.astype(BF16)

    qmax_s[...] = jnp.zeros(qmax_s.shape, F32)
    kmax_s[...] = jnp.zeros(kmax_s.shape, F32)
    vmax_s[...] = jnp.zeros(vmax_s.shape, F32)

    def proj_body(i, carry):
        r0 = pl.multiple_of(i * TP, TP)
        xb = x_v[pl.ds(r0, TP), :]
        qk = _dot(xb, wqk_s[...])
        qb = (qk[:, 0:768] * QSCALE).astype(BF16)
        kb = qk[:, 768:1536].astype(BF16)
        for t in range(6):
            q_s[t, pl.ds(r0, TP), :] = qb[:, t * 128:(t + 1) * 128]
            k_s[t, pl.ds(pl.multiple_of(i * (TP // 2), TP // 2), TP // 2), :] = pltpu.bitcast(
                kb[:, t * 128:(t + 1) * 128], U32)
        qa = jnp.abs(qb.astype(F32)).reshape(TP // 8, 8, 768)
        ka = jnp.abs(kb.astype(F32)).reshape(TP // 8, 8, 768)
        qmax_s[...] = jnp.maximum(qmax_s[...], jnp.max(qa, axis=0))
        kmax_s[...] = jnp.maximum(kmax_s[...], jnp.max(ka, axis=0))
        vg = _dot(wvt_s[...], xb, NT)
        v = vg[0:D].astype(BF16).astype(F32)
        vt_s[:, pl.ds(r0, TP)] = v
        va = jnp.abs(v).reshape(D // 8, 8, TP)
        vmax_s[...] = jnp.maximum(vmax_s[...], jnp.max(va, axis=0))
        gt_s[:, pl.ds(r0, TP)] = jax.nn.sigmoid(vg[D:D + 8])
        return carry

    lax.fori_loop(0, S // TP, proj_body, 0)

    qm1 = jnp.max(qmax_s[...], axis=0, keepdims=True)
    km1 = jnp.max(kmax_s[...], axis=0, keepdims=True)
    bound = DH * jnp.max(qm1 * km1)
    vmax = jnp.max(vmax_s[...])
    ok = jnp.logical_and(bound <= SAFE_LOG2, jnp.logical_and(vmax <= V_HI, vmax >= V_LO))
    flag_s[0] = ok.astype(jnp.int32)

    for i in range(3, 7):
        cps[i].wait()
    for h in range(H):
        t_s[h * DH:(h + 1) * DH, 0:DH] = wphi_v[h].astype(F32)
    tmat = jnp.where(_iota((D, 128), 1) < DH, t_s[...], 0.0).astype(BF16)
    bdt = []
    for n in range(5):
        lo, hi = RN[n]
        rows = _iota((hi - lo, 128), 0) + lo
        cols = _iota((hi - lo, 128), 1)
        sel = (rows % DH == cols).astype(BF16)
        full = _dot(sel, tmat[n * 128:(n + 1) * 128], NT)
        same = (rows // DH) == ((cols + n * 128) // DH)
        bdt.append(jnp.where(same, full, 0.0).astype(BF16))
    for j in range(2):
        parts = [_dot(bdt[n], wb_v[:, j * D + n * 128:j * D + (n + 1) * 128], NT) for n in range(5)]
        wbt_s[j * D:(j + 1) * D, :] = (_scatter_rn(parts) * LOG2E).astype(BF16)
    wbt_s[2 * D:3 * D, :] = wb_v[:, 2 * D:3 * D].T
    wot_s[:, 0:D] = woa_v[...].T
    wot_s[:, D:2 * D] = wob_v[...].T
    kvp_s[...] = jnp.zeros(kvp_s.shape, F32)
    kvn_s[...] = jnp.zeros(kvn_s.shape, F32)

    def linear_pass1(i):
        r0 = pl.multiple_of(i * TB, TB)
        xb = x_v[pl.ds(r0, TB), :]
        pr = _dot(wbt_s[...], xb, NT)
        qp, qn = _dual_softmax(pr[0:D])
        phiq_s[0:D // 2, pl.ds(r0, TB)] = pltpu.bitcast(qp.astype(BF16), U32)
        phiq_s[D // 2:D, pl.ds(r0, TB)] = pltpu.bitcast(qn.astype(BF16), U32)
        kp, kn = _dual_softmax(pr[D:2 * D])
        kp = kp.astype(BF16)
        kn = kn.astype(BF16)
        vb = pr[2 * D:3 * D].astype(BF16)
        ones = jnp.ones((16, TB), BF16)
        for n in range(5):
            lo, hi = RN[n]
            lhs = jnp.concatenate([vb[lo:hi], ones], axis=0)
            rows = hi - lo + 16
            kvp_s[n, 0:rows, :] += _dot(lhs, kp[n * 128:(n + 1) * 128], NT)
            kvn_s[n, 0:rows, :] += _dot(lhs, kn[n * 128:(n + 1) * 128], NT)

    def head_params(h):
        t = h // 6
        off = h * DH - jnp.minimum(t * 120, 512)
        return t, off

    def masked_q(t, off, qb):
        q = q_s[t, qb * TQ:(qb + 1) * TQ, :]
        lane = _iota((TQ, 128), 1)
        keep = jnp.logical_and(lane >= off, lane < off + DH)
        return jnp.where(keep, q.astype(F32), 0.0).astype(BF16)

    def v_rows(pair, hh, c0, width):
        base = pl.multiple_of(pair * (2 * DH) + 16 * hh, 8)
        v = vt_s[pl.ds(base, 24), c0:c0 + width]
        ones_row = 20 if hh == 0 else 0
        return jnp.where(_iota((24, width), 0) == ones_row, 1.0, v)

    def finish(pair, qb, acc0, acc1):
        o0 = acc0[0:DH] / acc0[DH:DH + 1]
        o1 = acc1[4:24] / acc1[0:1]
        base = pl.multiple_of(pair * (2 * DH), 8)
        at_s[pl.ds(base, 2 * DH), qb * TQ:(qb + 1) * TQ] = jnp.concatenate([o0, o1], axis=0)

    def attn_fast(i, carry):
        linear_pass1(i)
        units = [(qb, hh, c) for qb in range(NQ) for hh in range(HPI) for c in range(NC)]
        prm = [head_params(i * HPI + hh) for hh in range(HPI)]
        qms = {}
        accs = {}

        def pbuf(qb, hh):
            return pbufs[(qb * HPI + hh) % 4]

        def qk(u):
            qb, hh, c = u
            t, off = prm[hh]
            if (qb, hh) not in qms:
                qms[(qb, hh)] = masked_q(t, off, qb)
            kc = pltpu.bitcast(k_s[t, c * KC // 2:(c + 1) * KC // 2, :], BF16)
            p = jnp.exp2(_dot(kc, qms[(qb, hh)], NT)).astype(BF16)
            pbuf(qb, hh)[c * KC // 2:(c + 1) * KC // 2, :] = pltpu.bitcast(p, U32)

        def pv(u):
            qb, hh, c = u
            pc = pltpu.bitcast(pbuf(qb, hh)[c * KC // 2:(c + 1) * KC // 2, :], BF16)
            o = _dot(v_rows(i, hh, c * KC, KC), pc)
            accs[(qb, hh)] = o if c == 0 else accs[(qb, hh)] + o
            if c == NC - 1 and hh == HPI - 1:
                finish(i, qb, accs[(qb, 0)], accs[(qb, 1)])

        n = len(units)
        for k in range(n + LAG):
            if k < n:
                qk(units[k])
            if k >= LAG:
                pv(units[k - LAG])
        return carry

    def attn_slow(i, carry):
        linear_pass1(i)
        for qb in range(NQ):
            accs = []
            for hh in range(HPI):
                t, off = head_params(i * HPI + hh)
                kk = pltpu.bitcast(k_s[t], BF16)
                s_s[...] = _dot(kk, masked_q(t, off, qb), NT)
                s = s_s[...]
                m = jnp.max(s, axis=0, keepdims=True)
                p = jnp.exp2(s - m).astype(BF16)
                accs.append(_dot(v_rows(i, hh, 0, S), p))
            finish(i, qb, accs[0], accs[1])
        return carry

    @pl.when(flag_s[0] == 1)
    def _():
        lax.fori_loop(0, H // HPI, attn_fast, 0)

    @pl.when(flag_s[0] != 1)
    def _():
        lax.fori_loop(0, H // HPI, attn_slow, 0)

    lhs_p, lhs_n = [], []
    hrow = _iota((H, 128), 0)
    for n in range(5):
        lo, hi = RN[n]
        rows = _iota((hi - lo, 128), 0) + lo
        cols = _iota((hi - lo, 128), 1) + n * 128
        same = (rows // DH) == (cols // DH)
        head_of_row = jnp.where(hrow < H // 2, 2 * hrow, 2 * (hrow - H // 2) + 1)
        zsel = head_of_row == ((_iota((H, 128), 1) + n * 128) // DH)
        for src, dst in ((kvp_s, lhs_p), (kvn_s, lhs_n)):
            kv = jnp.where(same, src[n, 0:hi - lo, :], 0.0)
            z = jnp.where(zsel, jnp.broadcast_to(src[n, hi - lo:hi - lo + 1, :], (H, 128)), 0.0)
            dst.append(jnp.concatenate([kv, z], axis=0).astype(BF16))

    out_cps = []
    for j in range(S // TF):
        c0 = j * TF
        parts = []
        den = None
        for n in range(5):
            lo, hi = RN[n]
            wp = pltpu.bitcast(phiq_s[n * 64:(n + 1) * 64, c0:c0 + TF], BF16)
            wn = pltpu.bitcast(phiq_s[D // 2 + n * 64:D // 2 + (n + 1) * 64, c0:c0 + TF], BF16)
            r = _dot(lhs_p[n], wp) + _dot(lhs_n[n], wn)
            parts.append(r[0:hi - lo])
            dn = r[hi - lo:hi - lo + H]
            den = dn if den is None else den + dn
        num = _scatter_rn(parts)
        g = gt_s[0:1, c0:c0 + TF]
        rcp = (1.0 - g) / (den + 1e-6)
        is_a = _iota((2 * DH, TF), 0) < DH
        brows = []
        for pr in range(H // 2):
            sc = jnp.where(is_a, rcp[pr:pr + 1], rcp[H // 2 + pr:H // 2 + pr + 1])
            brows.append(num[pr * 2 * DH:(pr + 1) * 2 * DH] * sc)
        bt = jnp.concatenate(brows, axis=0).astype(BF16)
        at = (at_s[:, c0:c0 + TF] * g).astype(BF16)
        ab = jnp.concatenate([at, bt], axis=0)
        ot = _dot(wot_s[...], ab)
        out_v[c0:c0 + TF, :] = ot.T.astype(BF16)
        cp = pltpu.make_async_copy(out_v.at[c0:c0 + TF, :], out_hbm.at[0, c0:c0 + TF, :], out_sems.at[j])
        cp.start()
        out_cps.append(cp)
    for cp in out_cps:
        cp.wait()


@jax.jit
def pallas_gated_mix__mha_block__linear_kernel_hedgehog__prompt_kernel(
    A_x: jax.Array,
    A_wqkv: jax.Array,
    A_wo: jax.Array,
    B_x: jax.Array,
    B_wqkv: jax.Array,
    B_w_phi: jax.Array,
    B_wo: jax.Array,
    gate_w: jax.Array,
):
    del B_x
    any_spec = pl.BlockSpec(memory_space=pl.ANY)
    scratch = [
        pltpu.VMEM((S, D), BF16),
        pltpu.VMEM((D, 3 * D), BF16),
        pltpu.VMEM((D, D), BF16),
        pltpu.VMEM((D, 3 * D), BF16),
        pltpu.VMEM((H, DH, DH), BF16),
        pltpu.VMEM((D, D), BF16),
        pltpu.VMEM((1, D), BF16),
        pltpu.VMEM((S, D), BF16),
        pltpu.VMEM((D, 1536), BF16),
        pltpu.VMEM((D + 16, D), BF16),
        pltpu.VMEM((3 * D, D), BF16),
        pltpu.VMEM((D, 2 * D), BF16),
        pltpu.VMEM((D, 128), F32),
        pltpu.VMEM((6, S, 128), BF16),
        pltpu.VMEM((6, S // 2, 128), U32),
        pltpu.VMEM((D, S), F32),
        pltpu.VMEM((8, S), F32),
        pltpu.VMEM((D, S), F32),
        pltpu.VMEM((8, 768), F32),
        pltpu.VMEM((8, 768), F32),
        pltpu.VMEM((8, TP), F32),
        pltpu.VMEM((D, S), U32),
        pltpu.VMEM((5, 176, 128), F32),
        pltpu.VMEM((5, 176, 128), F32),
        pltpu.VMEM((S, TQ), F32),
        pltpu.VMEM((S // 2, TQ), U32),
        pltpu.VMEM((S // 2, TQ), U32),
        pltpu.VMEM((S // 2, TQ), U32),
        pltpu.VMEM((S // 2, TQ), U32),
        pltpu.SMEM((1,), jnp.int32),
        pltpu.SemaphoreType.DMA((7,)),
        pltpu.SemaphoreType.DMA((S // TF,)),
    ]
    return pl.pallas_call(
        _kernel,
        out_shape=jax.ShapeDtypeStruct((1, S, D), BF16),
        in_specs=[any_spec] * 7,
        out_specs=any_spec,
        scratch_shapes=scratch,
        compiler_params=pltpu.CompilerParams(vmem_limit_bytes=110 * 1024 * 1024),
    )(A_x, A_wqkv, A_wo, B_wqkv, B_w_phi, B_wo, gate_w.reshape(1, D))
```

```python
import math

import jax
import jax.numpy as jnp
from jax import lax
import jax.experimental.pallas as pl
import jax.experimental.pallas.tpu as pltpu

F32 = jnp.float32
BF16 = jnp.bfloat16
U32 = jnp.uint32

S = 2048
D = 640
H = 32
DH = 20
LOG2E = math.log2(math.e)
QSCALE = (DH ** -0.5) * LOG2E

WIN = (0, 120, 240, 360, 480, 512)
RN = ((0, 144), (112, 272), (240, 400), (368, 528), (496, 640))

TQ = 512
KC = 128
NQ = S // TQ
NC = S // KC
TB = 128
NV = 2
PRO_UNITS = (3, 3, 2)
GEN_K = 64
GEN_Q = 512
TP = 256
FINAL_UNROLL = 1
TF = 512

SAFE_LOG2 = 80.0
V_HI = 2.0 ** 30
V_LO = 2.0 ** -16

NN = (((1,), (0,)), ((), ()))
NT = (((1,), (1,)), ((), ()))


def _dot(a, b, dims=NN):
    return lax.dot_general(a, b, dims, preferred_element_type=F32)


def _iota(shape, dim):
    return lax.broadcasted_iota(jnp.int32, shape, dim)


def _recip(x):
    r = pl.reciprocal(x, approx=True)
    return r * (2.0 - x * r)


def _dual_softmax(x):
    rows, t = x.shape
    x3 = x.reshape(rows // (2 * DH), 2 * DH, t)
    lo = _iota((rows // (2 * DH), 8, t), 1) < 4

    def split(v):
        return v[:, 0:8], v[:, 8:16], v[:, 16:24], v[:, 24:32], v[:, 32:40]

    def seg(comb, red, fill, v):
        v0, v1, v2, v3, v4 = split(v)
        ra = comb(comb(v0, v1), jnp.where(lo, v2, fill))
        rb = comb(comb(v3, v4), jnp.where(lo, fill, v2))
        return red(ra, axis=1, keepdims=True), red(rb, axis=1, keepdims=True)

    def apply(fn, v, ra, rb):
        v0, v1, v2, v3, v4 = split(v)
        return jnp.concatenate(
            [fn(v0, ra), fn(v1, ra), fn(v2, jnp.where(lo, ra, rb)), fn(v3, rb), fn(v4, rb)], axis=1)

    inf = jnp.float32(jnp.inf)
    ep = apply(lambda v, m: jnp.exp2(v - m), x3, *seg(jnp.maximum, jnp.max, -inf, x3))
    en = apply(lambda v, m: jnp.exp2(m - v), x3, *seg(jnp.minimum, jnp.min, inf, x3))
    out = []
    for e in (ep, en):
        sa, sb = seg(jnp.add, jnp.sum, 0.0, e)
        out.append(apply(jnp.multiply, e, _recip(sa), _recip(sb)).reshape(rows, t))
    return out


def _scatter_rn(parts):
    pieces = []
    for n in range(5):
        lo, hi = RN[n]
        start = lo if n == 0 else RN[n - 1][1]
        stop = hi if n == 4 else RN[n + 1][0]
        pieces.append(parts[n][start - lo:stop - lo])
        if n < 4:
            nlo = RN[n + 1][0]
            pieces.append(parts[n][nlo - lo:hi - lo] + parts[n + 1][0:hi - nlo])
    return jnp.concatenate(pieces, axis=0)


_SCRATCH = dict(
    p_s=pltpu.VMEM((2 * NQ * S // 2, TQ), U32),
    q_s=pltpu.VMEM((6, S, 128), BF16),
    k_s=pltpu.VMEM((6, S // 2, 128), U32),
    vt_s=pltpu.VMEM((D, S), F32),
    at_s=pltpu.VMEM((D, S), F32),
    kb0_s=pltpu.VMEM((NV * DH * KC, 128), F32),
    kb1_s=pltpu.VMEM((NV * DH * KC, 128), F32),
    qb0_s=pltpu.VMEM((DH * 8, S), F32),
    qb1_s=pltpu.VMEM((DH * 8, S), F32),
    qt_s=pltpu.VMEM((768, S), F32),
    phiq_s=pltpu.VMEM((D, S), U32),
    x_v=pltpu.VMEM((S, D), BF16),
    out_v=pltpu.VMEM((S, D), BF16),
    s_s=pltpu.VMEM((S, TQ), F32),
    kr0_s=pltpu.VMEM((256, 128), F32),
    kr1_s=pltpu.VMEM((256, 128), F32),
    pr0_s=pltpu.VMEM((2048, TB), F32),
    pr1_s=pltpu.VMEM((2048, TB), F32),
    phik0_s=pltpu.VMEM((1024, TB), U32),
    phik1_s=pltpu.VMEM((1024, TB), U32),
    wbt_s=pltpu.VMEM((1024, D), U32),
    wa_v=pltpu.VMEM((D, 3 * D), BF16),
    wb_v=pltpu.VMEM((D, 3 * D), BF16),
    woa_v=pltpu.VMEM((D, D), BF16),
    wob_v=pltpu.VMEM((D, D), BF16),
    wvt_s=pltpu.VMEM((D + 16, D), BF16),
    wot_s=pltpu.VMEM((D, 2 * D), BF16),
    kvp_s=pltpu.VMEM((5, 176, 128), F32),
    kvn_s=pltpu.VMEM((5, 176, 128), F32),
    lhs_s=pltpu.VMEM((5, 96, 256), U32),
    bdt_s=pltpu.VMEM((5, 80, 128), U32),
    gt_s=pltpu.VMEM((8, S), F32),
    qmax_s=pltpu.VMEM((8, D), F32),
    kmax_s=pltpu.VMEM((8, D), F32),
    vmax_s=pltpu.VMEM((8, TP), F32),
    wphi_v=pltpu.VMEM((DH, DH, H), BF16),
    gw_v=pltpu.VMEM((D,), BF16),
    flag_s=pltpu.SMEM((1,), jnp.int32),
    in_sems=pltpu.SemaphoreType.DMA((8,)),
    x_sems=pltpu.SemaphoreType.DMA((S // TP,)),
    out_sems=pltpu.SemaphoreType.DMA((S // TF,)),
)


def _kernel(x_hbm, wa_hbm, woa_hbm, wb_hbm, wphi_hbm, wob_hbm, gw_hbm, out_hbm, *scratch):
    sc = dict(zip(_SCRATCH, scratch, strict=True))
    (x_v, wa_v, woa_v, wb_v, wphi_v, wob_v, gw_v, out_v, wvt_s, wbt_s, wot_s,
     q_s, k_s, vt_s, gt_s, at_s, qmax_s, kmax_s, vmax_s, phiq_s, kvp_s, kvn_s, lhs_s,
     s_s, p_s, qt_s, kb0_s, kb1_s, qb0_s, qb1_s, kr0_s, kr1_s, flag_s, in_sems, x_sems, out_sems) = (
        sc[n] for n in (
            'x_v wa_v woa_v wb_v wphi_v wob_v gw_v out_v wvt_s wbt_s wot_s '
            'q_s k_s vt_s gt_s at_s qmax_s kmax_s vmax_s phiq_s kvp_s kvn_s lhs_s '
            's_s p_s qt_s kb0_s kb1_s qb0_s qb1_s kr0_s kr1_s flag_s in_sems x_sems out_sems').split())
    kb_s, qb_s, kr_s = (kb0_s, kb1_s), (qb0_s, qb1_s), (kr0_s, kr1_s)
    pr_s, phik_s = (sc['pr0_s'], sc['pr1_s']), (sc['phik0_s'], sc['phik1_s'])
    bdt_s = sc['bdt_s']
    def x_copy(i):
        r0 = pl.multiple_of(i * TP, TP)
        return pltpu.make_async_copy(x_hbm.at[0, pl.ds(r0, TP), :], x_v.at[pl.ds(r0, TP), :], x_sems.at[i])

    cps = [pltpu.make_async_copy(src, dst, in_sems.at[i]) for i, (src, dst) in enumerate(
        ((wa_hbm.at[:, 0:D], wa_v.at[:, 0:D]), (gw_hbm, gw_v), (wb_hbm, wb_v), (wphi_hbm, wphi_v),
         (woa_hbm, woa_v), (wob_hbm, wob_v), (wa_hbm.at[:, 2 * D:3 * D], wa_v.at[:, 2 * D:3 * D]),
         (wa_hbm.at[:, D:2 * D], wa_v.at[:, D:2 * D])))]
    cps[3].start()
    x_copy(0).start()
    cps[7].start()

    def store_q(i, q):
        r0 = pl.multiple_of(i * TP, TP)
        qb = (q * QSCALE).astype(BF16)
        for t in range(6):
            qw = qb[:, WIN[t]:WIN[t] + 128]
            q_s[t, pl.ds(r0, TP), :] = qw
            qt_s[t * 128:(t + 1) * 128, pl.ds(r0, TP)] = qw.astype(F32).T
        qa = jnp.abs(qb.astype(F32)).reshape(TP // 8, 8, D)
        qmax_s[...] = jnp.maximum(qmax_s[...], jnp.max(qa, axis=0))

    def store_k(i, k):
        kb = k.astype(BF16)
        for t in range(6):
            k_s[t, pl.ds(pl.multiple_of(i * (TP // 2), TP // 2), TP // 2), :] = pltpu.bitcast(
                kb[:, WIN[t]:WIN[t] + 128], U32)
        ka = jnp.abs(kb.astype(F32)).reshape(TP // 8, 8, D)
        kmax_s[...] = jnp.maximum(kmax_s[...], jnp.max(ka, axis=0))

    def proj_v(i):
        r0 = pl.multiple_of(i * TP, TP)
        vg = _dot(wvt_s[...], x_v[pl.ds(r0, TP), :], NT)
        v = vg[0:D].astype(BF16).astype(F32)
        vt_s[:, pl.ds(r0, TP)] = v
        va = jnp.abs(v).reshape(D // 8, 8, TP)
        vmax_s[...] = jnp.maximum(vmax_s[...], jnp.max(va, axis=0))
        gt_s[:, pl.ds(r0, TP)] = jax.nn.sigmoid(vg[D:D + 8])

    def proj_block(i):
        r0 = pl.multiple_of(i * TP, TP)
        qk = _dot(x_v[pl.ds(r0, TP), :], wa_v[:, 0:2 * D])
        store_q(i, qk[:, 0:D])
        store_k(i, qk[:, D:2 * D])
        proj_v(i)

    def proj_body(j, carry):
        x_copy(2 * j + 1).wait()
        x_copy(2 * j + 2).wait()
        proj_block(2 * j + 1)
        proj_block(2 * j + 2)
        return carry

    for ref in (kvp_s, kvn_s, qmax_s, kmax_s, vmax_s, pr_s[1]):
        ref[...] = jnp.zeros(ref.shape, F32)
    cps[3].wait()
    cps[0].start()
    cps[6].start()
    cps[1].start()
    mcat = jnp.concatenate([wphi_v[d].astype(F32) for d in range(DH)], axis=1)
    mcat = jnp.concatenate([mcat, jnp.zeros((12, D), F32)], axis=0).astype(BF16)
    src = _iota((D, D), 0)
    perm = (_iota((D, D), 1) == (src % H) * DH + src // H).astype(BF16)
    gmat = _dot(mcat, perm).astype(BF16)
    for n in range(5):
        lo, hi = RN[n]
        rows = _iota((hi - lo, 32), 0) + lo
        sel = (rows % DH == _iota((hi - lo, 32), 1)).astype(BF16)
        full = _dot(sel, gmat[:, n * 128:(n + 1) * 128])
        same = ((_iota((hi - lo, 128), 0) + lo) // DH) == ((_iota((hi - lo, 128), 1) + n * 128) // DH)
        bdt_s[n, 0:(hi - lo) // 2, :] = pltpu.bitcast(jnp.where(same, full, 0.0).astype(BF16), U32)

    x_copy(0).wait()
    cps[7].wait()
    store_k(0, _dot(x_v[0:TP, :], wa_v[:, D:2 * D]))
    cps[0].wait()
    cps[6].wait()
    cps[1].wait()
    for i in range(1, S // TP):
        x_copy(i).start()
    store_q(0, _dot(x_v[0:TP, :], wa_v[:, 0:D]))
    wvt_s[0:D, :] = wa_v[:, 2 * D:3 * D].T
    gw_rows = jnp.where(_iota((16, D), 0) == 0, jnp.broadcast_to(gw_v[...].astype(F32).reshape(1, D), (16, D)), 0.0)
    wvt_s[D:D + 16, :] = gw_rows.astype(BF16)
    proj_v(0)
    for j in (2, 4, 5):
        cps[j].start()
    lax.fori_loop(0, (S // TP - 2) // 2, proj_body, 0)

    rt = {}

    def runtime_zero():
        rt['zero'] = pl.multiple_of(flag_s[0] >> 1, 8192)
        rt['never'] = _iota((8, 128), 0) < rt['zero']
        return rt['zero']

    def after(gate, x):
        if gate is None:
            return x
        r, c = x.shape
        never = rt['never']
        g = gate if c == 128 else jnp.concatenate([gate] * (c // 128), axis=1)
        m = never if c == 128 else jnp.concatenate([never] * (c // 128), axis=1)
        return jnp.where(m, g, x.reshape(r // 8, 8, c)).reshape(r, c)

    def rsl(z, r0, n):
        return slice(r0, r0 + n) if z is None else pl.ds(z + r0, n)

    def linear_pass1_tasks(i, buf, z=None, live=1.0):
        r0 = pl.multiple_of(i * TB, TB)
        slab = 4 * DH
        pr, phik = pr_s[buf], phik_s[buf]

        def project(m):
            xb = x_v[pl.ds(r0, TB), :]
            w = pltpu.bitcast(wbt_s[m * D // 2:(m + 1) * D // 2, :], BF16)
            pr[m * D:(m + 1) * D, :] = _dot(w, xb, NT)

        def load_slab(r, gate):
            return after(gate, pr[rsl(z, r, slab), :])

        def q_feat(j, gate):
            qp, qn = _dual_softmax(load_slab(j * slab, gate))
            h0 = j * slab // 2
            phiq_s[h0:h0 + slab // 2, pl.ds(r0, TB)] = pltpu.bitcast(qp.astype(BF16), U32)
            phiq_s[D // 2 + h0:D // 2 + h0 + slab // 2, pl.ds(r0, TB)] = pltpu.bitcast(qn.astype(BF16), U32)

        def k_feat(j, gate):
            kp, kn = _dual_softmax(load_slab(D + j * slab, gate))
            h0 = j * slab // 2
            phik[h0:h0 + slab // 2, :] = pltpu.bitcast(kp.astype(BF16), U32)
            phik[D // 2 + h0:D // 2 + h0 + slab // 2, :] = pltpu.bitcast(kn.astype(BF16), U32)

        def kv(n, live):
            lo, hi = RN[n]
            vb = pr[rsl(z, 2 * D + lo, hi - lo), :].astype(BF16)
            lhs = jnp.concatenate([vb, jnp.full((16, TB), live, F32).astype(BF16)], axis=0)
            nrows = hi - lo + 16
            kp = pltpu.bitcast(phik[rsl(z, n * 64, 64), :], BF16)
            kn = pltpu.bitcast(phik[rsl(z, D // 2 + n * 64, 64), :], BF16)
            res = _dot(lhs, jnp.concatenate([kp, kn], axis=0), NT)
            kvp_s[n, 0:nrows, :] += res[:, 0:128]
            kvn_s[n, 0:nrows, :] += res[:, 128:256]

        kfs = [lambda gate, j=j: k_feat(j, gate) for j in range(D // slab)]
        qfs = [lambda gate, j=j: q_feat(j, gate) for j in range(D // slab)]
        kvs = [lambda n=n, live=live: kv(n, live) for n in range(5)]
        return project, kfs, kvs, qfs

    def head_params(h):
        t = h // 6
        off = h * DH - jnp.minimum(t * 120, 512)
        return t, off

    def masked_q(t, off, q0):
        q = q_s[t, pl.ds(q0, TQ), :]
        lane = _iota((TQ, 128), 1)
        keep = jnp.logical_and(lane >= off, lane < off + DH)
        return jnp.where(keep, q.astype(F32), 0.0).astype(BF16)

    def v_rows(pair, hh, c0, width):
        base = pl.multiple_of(pair * (2 * DH) + 16 * hh, 8)
        v = vt_s[pl.ds(base, 24), pl.ds(c0, width)]
        ones_row = 20 if hh == 0 else 0
        return jnp.where(_iota((24, width), 0) == ones_row, 1.0, v)

    def finish(pair, hh, q0, acc):
        base = pl.multiple_of(pair * (2 * DH) + 16 * hh, 8)
        if hh == 0:
            at_s[pl.ds(base, 24), pl.ds(q0, TQ)] = acc * _recip(acc[DH:DH + 1])
        else:
            old = at_s[pl.ds(base, 24), pl.ds(q0, TQ)]
            at_s[pl.ds(base, 24), pl.ds(q0, TQ)] = jnp.where(_iota((24, TQ), 0) < 4, old, acc * _recip(acc[0:1]))

    def qk_unit(t, qm, prow, c, n=1):
        kc = pltpu.bitcast(k_s[t, c * KC // 2:(c + n) * KC // 2, :], BF16)
        s = _dot(kc, qm, NT)
        p_s[pl.ds(prow + c * (KC // 2), n * KC // 2), :] = pltpu.bitcast(jnp.exp2(s).astype(BF16), U32)
        return s

    def pv_unit(pair, hh, prow, c, n=1):
        pc = pltpu.bitcast(p_s[pl.ds(prow + c * (KC // 2), n * KC // 2), :], BF16)
        return _dot(v_rows(pair, hh, c * KC, n * KC), pc)

    def bcast_tasks(slot, h, z=None):
        t, off = head_params(h)
        kb, qb = kb_s[slot], qb_s[slot]

        def prep(part, gate):
            r0 = part * 64
            kf = pltpu.bitcast(k_s[t, r0 // 2:(r0 + 64) // 2, :], BF16).astype(F32)
            kr_s[slot][r0:r0 + 64, :] = pltpu.roll(after(gate, kf), (128 - off) % 128, 1)

        def kstep(d, part, gate):
            r0 = part * GEN_K
            kr = after(gate, kr_s[slot][rsl(z, r0, GEN_K), :])
            o0 = ((r0 // KC) * DH + d) * KC + r0 % KC
            kb[o0:o0 + GEN_K, :] = jnp.broadcast_to(kr[:, d:d + 1], (GEN_K, 128))

        def qstep(d, part, gate):
            c0 = part * GEN_Q
            row = qt_s[pl.ds(t * 128 + off + d, 1), c0:c0 + GEN_Q]
            if gate is not None:
                row = jnp.where(rt['never'][0:1, 0:1], jnp.concatenate([gate[0:1]] * (GEN_Q // 128), axis=1), row)
            qb[d * 8:(d + 1) * 8, c0:c0 + GEN_Q] = jnp.broadcast_to(row, (8, GEN_Q))

        tasks = [lambda gate, part=part: prep(part, gate) for part in range(NV * KC // 64)]
        nk, nq = NV * KC // GEN_K, S // GEN_Q
        for d in range(DH):
            for part in range(max(nk, nq)):
                if part < nk:
                    tasks.append(lambda gate, d=d, part=part: kstep(d, part, gate))
                if part < nq:
                    tasks.append(lambda gate, d=d, part=part: qstep(d, part, gate))
        return tasks

    def vpu_scores(slot, qb, prow, z):
        kb, qbr = kb_s[slot], qb_s[slot]
        nl = TQ // 128
        for vc in range(NV):
            for g0 in range(0, KC // 8, 2):
                acc = [[None] * nl for _ in range(2)]
                for d in range(DH):
                    r0 = (vc * DH + d) * KC + g0 * 8
                    gate = yield
                    ks = [after(gate, kb[rsl(z, r0 + r * 8, 8), :]) for r in range(2)]
                    qs = [qbr[rsl(z, d * 8, 8), qb * TQ + j * 128:qb * TQ + (j + 1) * 128] for j in range(nl)]
                    for r in range(2):
                        for j in range(nl):
                            prod = ks[r] * qs[j]
                            acc[r][j] = prod if acc[r][j] is None else acc[r][j] + prod
                sc = jnp.concatenate([jnp.concatenate(acc[r], axis=1) for r in range(2)], axis=0)
                p0 = prow + vc * (KC // 2) + g0 * 4
                p_s[p0:p0 + 8, :] = pltpu.bitcast(jnp.exp2(sc).astype(BF16), U32)
        while True:
            yield

    def attn_prologue(b, carry):
        z = runtime_zero()
        hh = b // NQ
        qb = b % NQ
        t, off = head_params(hh)
        qm = masked_q(t, off, pl.multiple_of(qb * TQ, TQ))
        prow = pl.multiple_of(b * (S // 2), S // 2)
        units = iter(range(NC))

        def unit(tasks):
            s = qk_unit(t, qm, prow, next(units))
            for n, task in enumerate(tasks):
                r = (n * (KC // 8)) // len(tasks)
                task(s[r * 8:(r + 1) * 8, 0:128])

        for half in range(2):
            project = linear_pass1_tasks(2 * b + half, half, z)[0]
            live = 1.0 if half == 1 else jnp.where(b > 0, 1.0, 0.0)
            _, kfs, kvs, qfs = linear_pass1_tasks(jnp.maximum(2 * b + half - 1, 0), 1 - half, z, live)
            tasks = kfs + qfs
            k = 0
            for g, m in enumerate((1, 2, 0)):
                project(m)
                for u in range(PRO_UNITS[g]):
                    unit(tasks[2 * k:2 * k + 2])
                    if k >= 4:
                        kvs[k - 4]()
                    k += 1
            kvs[4]()
        return carry

    def wo_task(j, gate):
        src = (woa_v, wob_v)[j // 5]
        c = j % 5
        w = src[:, c * 128:(c + 1) * 128]
        if gate is not None:
            w = after(gate, w.astype(F32)).astype(BF16)
        wot_s[c * 128:(c + 1) * 128, (j // 5) * D:(j // 5 + 1) * D] = w.T

    def attn_epilogue():
        pair = H // 2 - 1
        runtime_zero()
        _, kfs, kvs, qfs = linear_pass1_tasks(H // 2 - 1, 1)
        tasks = kfs + [lambda gate, kv=kv: kv() for kv in kvs] + qfs + [
            lambda gate, j=j: wo_task(j, gate) for j in range(10)]
        k = 0
        for hh in range(2):
            for qb in range(NQ):
                prow = (hh * NQ + qb) * (S // 2)
                acc = None
                for c in range(NC):
                    o = pv_unit(pair, hh, prow, c)
                    acc = o if acc is None else acc + o
                    if k % 4 == 0 and k // 4 < len(tasks):
                        tasks[k // 4](o[0:8, 0:128])
                    k += 1
                finish(pair, hh, qb * TQ, acc)

    def attn_fast(i, carry):
        z = runtime_zero()
        prm = [head_params((i + 1) * 2 + hh) for hh in range(2)]
        gens = [bcast_tasks(1, (i + 1) * 2 + 1, z), bcast_tasks(0, jnp.minimum((i + 2) * 2, H - 1), z)]
        assert NV == 2
        nsteps = NV * (KC // 16) * DH
        for hh in range(2):
            t, off = prm[hh]
            gen = gens[hh]
            for qb in range(NQ):
                prow = (hh * NQ + qb) * (S // 2)
                qm = masked_q(t, off, qb * TQ)
                vs = vpu_scores(hh, qb, prow, z)
                next(vs)
                acc = pv_unit(i, hh, prow, 0) + pv_unit(i, hh, prow, 1)
                done = 0
                for c in range(NV, NC):
                    acc = acc + pv_unit(i, hh, prow, c)
                    s = qk_unit(t, qm, prow, c)
                    gidx = [0]
                    gates = {}

                    def gate(n, s=s, gidx=gidx, gates=gates):
                        r = ((2 * gidx[0] + 1) * (KC // 8)) // (2 * n)
                        gidx[0] += 1
                        if r not in gates:
                            gates[r] = s[r * 8:(r + 1) * 8, 0:128]
                        return gates[r]

                    tgt = (c - NV + 1) * nsteps // (NC - NV)
                    tot = NQ * (NC - NV) - 3
                    kh = qb * (NC - NV) + c - NV
                    extra = gen[kh * len(gen) // tot:(kh + 1) * len(gen) // tot]
                    n = tgt - done + len(extra)
                    todo = [vs.send] * (tgt - done)
                    nst = len(todo)
                    for q, task in enumerate(extra):
                        todo.insert((q * nst) // len(extra) + q, task)
                    for task in todo:
                        task(gate(n))
                    done = tgt
                finish(i, hh, qb * TQ, acc)
        return carry

    def attn_slow(i, carry):
        sc = 256

        def block(qb, carry2):
            q0 = pl.multiple_of(qb * TQ, TQ)
            for hh in range(2):
                t, off = head_params(i * 2 + hh)
                qm = masked_q(t, off, q0)

                def scores(c, m8, t=t, qm=qm):
                    kc = pltpu.bitcast(k_s[t, pl.ds(pl.multiple_of(c * (sc // 2), sc // 2), sc // 2), :], BF16)
                    s = _dot(kc, qm, NT)
                    s_s[pl.ds(pl.multiple_of(c * sc, sc), sc), :] = s
                    return jnp.maximum(m8, jnp.max(s.reshape(sc // 8, 8, TQ), axis=0))

                m8 = lax.fori_loop(0, S // sc, scores, jnp.full((8, TQ), -jnp.inf, F32))
                m = jnp.max(m8, axis=0, keepdims=True)

                def weigh(c, acc, hh=hh, m=m):
                    c0 = pl.multiple_of(c * sc, sc)
                    p = jnp.exp2(s_s[pl.ds(c0, sc), :] - m).astype(BF16)
                    return acc + _dot(v_rows(i, hh, c0, sc), p)

                finish(i, hh, q0, lax.fori_loop(0, S // sc, weigh, jnp.zeros((24, TQ), F32)))
            return carry2

        lax.fori_loop(0, NQ, block, 0)
        return carry

    for i in (2, 4, 5):
        cps[i].wait()
    x_copy(S // TP - 1).wait()
    proj_block(S // TP - 1)

    qm1 = jnp.max(qmax_s[...], axis=0, keepdims=True)
    km1 = jnp.max(kmax_s[...], axis=0, keepdims=True)
    seg = (_iota((D, 128), 0) // DH == _iota((D, 128), 1)).astype(BF16)
    per_head = _dot(jnp.broadcast_to(qm1 * km1, (8, D)), seg)
    bound = 1.02 * jnp.max(per_head)
    vmax = jnp.max(vmax_s[...])
    ok = jnp.logical_and(bound <= SAFE_LOG2, jnp.logical_and(vmax <= V_HI, vmax >= V_LO))
    flag_s[0] = ok.astype(jnp.int32)

    for j in range(2):
        parts = [_dot(pltpu.bitcast(bdt_s[n, 0:(RN[n][1] - RN[n][0]) // 2, :], BF16),
                      wb_v[:, j * D + n * 128:j * D + (n + 1) * 128], NT) for n in range(5)]
        wbt_s[j * D // 2:(j + 1) * D // 2, :] = pltpu.bitcast((_scatter_rn(parts) * LOG2E).astype(BF16), U32)
    wbt_s[D:3 * D // 2, :] = pltpu.bitcast(wb_v[:, 2 * D:3 * D].T, U32)

    for task in bcast_tasks(0, 2):
        task(None)


    lax.fori_loop(0, 2 * NQ, attn_prologue, 0)

    @pl.when(flag_s[0] == 1)
    def _():
        lax.fori_loop(0, H // 2 - 1, attn_fast, 0)

    attn_epilogue()
    hrow = _iota((H, 128), 0)
    for n in range(5):
        lo, hi = RN[n]
        rows = _iota((hi - lo, 128), 0) + lo
        cols = _iota((hi - lo, 128), 1) + n * 128
        same = (rows // DH) == (cols // DH)
        head_of_row = jnp.where(hrow < H // 2, 2 * hrow, 2 * (hrow - H // 2) + 1)
        zsel = head_of_row == ((_iota((H, 128), 1) + n * 128) // DH)
        for sgn, src in enumerate((kvp_s, kvn_s)):
            kv = jnp.where(same, src[n, 0:hi - lo, :], 0.0)
            z = jnp.where(zsel, jnp.broadcast_to(src[n, hi - lo:hi - lo + 1, :], (H, 128)), 0.0)
            lhs = jnp.concatenate([kv, z], axis=0).astype(BF16)
            lhs_s[n, 0:(hi - lo + H) // 2, sgn * 128:(sgn + 1) * 128] = pltpu.bitcast(lhs, U32)

    @pl.when(flag_s[0] != 1)
    def _():
        lax.fori_loop(0, H // 2, attn_slow, 0)

    def out_copy(j):
        c0 = pl.multiple_of(j * TF, TF)
        return pltpu.make_async_copy(out_v.at[pl.ds(c0, TF), :], out_hbm.at[0, pl.ds(c0, TF), :], out_sems.at[j])

    def final_block(j):
        c0 = pl.multiple_of(j * TF, TF)
        parts = []
        den = None
        for n in range(5):
            lo, hi = RN[n]
            nr = (hi - lo + H) // 2
            wp = pltpu.bitcast(phiq_s[n * 64:(n + 1) * 64, pl.ds(c0, TF)], BF16)
            wn = pltpu.bitcast(phiq_s[D // 2 + n * 64:D // 2 + (n + 1) * 64, pl.ds(c0, TF)], BF16)
            r = _dot(pltpu.bitcast(lhs_s[n, 0:nr, :], BF16), jnp.concatenate([wp, wn], axis=0))
            parts.append(r[0:hi - lo])
            dn = r[hi - lo:hi - lo + H]
            den = dn if den is None else den + dn
        num = _scatter_rn(parts)
        g = gt_s[0:1, pl.ds(c0, TF)]
        rcp = (1.0 - g) / (den + 1e-6)
        is_a = _iota((2 * DH, TF), 0) < DH
        brows = []
        for pr in range(H // 2):
            sc = jnp.where(is_a, rcp[pr:pr + 1], rcp[H // 2 + pr:H // 2 + pr + 1])
            brows.append(num[pr * 2 * DH:(pr + 1) * 2 * DH] * sc)
        bt = jnp.concatenate(brows, axis=0).astype(BF16)
        at = (at_s[:, pl.ds(c0, TF)] * g).astype(BF16)
        ab = jnp.concatenate([at, bt], axis=0)
        ot = _dot(wot_s[...], ab)
        out_v[pl.ds(c0, TF), :] = ot.T.astype(BF16)
        out_copy(j).start()

    def final_body(j, carry):
        for u in range(FINAL_UNROLL):
            final_block(j * FINAL_UNROLL + u)
        return carry

    lax.fori_loop(0, S // TF // FINAL_UNROLL, final_body, 0)
    for j in range(S // TF):
        out_copy(j).wait()


@jax.jit
def pallas_gated_mix__mha_block__linear_kernel_hedgehog__prompt_kernel(
    A_x: jax.Array,
    A_wqkv: jax.Array,
    A_wo: jax.Array,
    B_x: jax.Array,
    B_wqkv: jax.Array,
    B_w_phi: jax.Array,
    B_wo: jax.Array,
    gate_w: jax.Array,
):
    del B_x
    any_spec = pl.BlockSpec(memory_space=pl.ANY)
    return pl.pallas_call(
        _kernel,
        out_shape=jax.ShapeDtypeStruct((1, S, D), BF16),
        in_specs=[any_spec] * 7,
        out_specs=any_spec,
        scratch_shapes=list(_SCRATCH.values()),
        compiler_params=pltpu.CompilerParams(vmem_limit_bytes=110 * 1024 * 1024),
    )(A_x, A_wqkv, A_wo, B_wqkv, B_w_phi.transpose(1, 2, 0), B_wo, gate_w)
```
